```python
import os as _os
_os.environ.setdefault("JAX_PLATFORMS", "cpu")
import jax
import jax.numpy as jnp

def _softmax(x, axis=-1):
    return jax.nn.softmax(x, axis=axis)
def _gelu(x):
    return jax.nn.gelu(x, approximate=True)
def _silu(x):
    return jax.nn.silu(x)
def _sigmoid(x):
    return jax.nn.sigmoid(x)
def _layernorm(x, axis=-1, eps=1e-5):
    m = jnp.mean(x, axis=axis, keepdims=True)
    v = jnp.var(x, axis=axis, keepdims=True)
    return (x - m) / jnp.sqrt(v + eps)
def _scatter_add(tgt, idx, src, axis=0):
    return tgt.at[idx].add(src)
def _segment_sum(src, seg, n):
    return jax.ops.segment_sum(src, seg, n)
class _Rng:
    def __init__(self, key):
        self._k = key
    def _next(self):
        self._k, sub = jax.random.split(self._k)
        return sub
    def normal(self, shape):
        return jax.random.normal(self._next(), shape, dtype=jnp.bfloat16)
    def randint(self, lo, hi, shape):
        return jax.random.randint(self._next(), shape, lo, hi, dtype=jnp.int32)
    def uniform(self, shape, lo=0.0, hi=1.0):
        return jax.random.uniform(self._next(), shape, jnp.bfloat16, lo, hi)
    def permutation(self, n):
        return jax.random.permutation(self._next(), n)


kernel_name = 'gated_mix__sliding_block__dense_activation_silu__prompt'

def setup_inputs():
    _rng = _Rng(jax.random.key(int.from_bytes(__import__("os").urandom(4), "little")))
    _w = (lambda a: (lambda t: t.astype(jnp.bfloat16) if jnp.issubdtype(t.dtype, jnp.floating) else t)(jnp.asarray(a)))
    def _A_setup():
        B, S, D = 1, 2048, 640
        return {
            "x": _w((lambda *s: _rng.normal(s) * 0.05)(B, S, D)),
            "wqkv": _w((lambda *s: _rng.normal(s) * 0.4)(D, 3 * D)),
            "wo": _w((lambda *s: _rng.normal(s) * 0.05)(D, D)),
        }
    _A_in = _A_setup()

    def _B_setup():
        B, S, D, F = 1, 2048, 640, 1536
        return {
            "x": _w((lambda *s: _rng.normal(s) * 0.05)(B, S, D)),
            "w1": _w((lambda *s: _rng.normal(s) * 1.6)(D, F) * (D ** -0.5)),
            "w2": _w((lambda *s: _rng.normal(s) * 1.6)(F, D) * (F ** -0.5)),
        }
    _B_in = _B_setup()

    return {
        "A_x": _A_in["x"],
        "A_wqkv": _A_in["wqkv"],
        "A_wo": _A_in["wo"],
        "B_x": _B_in["x"],
        "B_w1": _B_in["w1"],
        "B_w2": _B_in["w2"],
        "gate_w": _w((lambda *s: _rng.normal(s) * 0.05)(640) * 16.0),
    }

def reference(A_x, A_wqkv, A_wo, B_x, B_w1, B_w2, gate_w):
    def _A_ref(x, wqkv, wo):
        B, S, D = x.shape
        H = 32; Dh = D // H; W = 256
        qkv = (lambda x, *d: x.transpose(*d))((x @ wqkv).reshape(B, S, 3, H, Dh), 2, 0, 3, 1, 4)
        q, k, v = qkv[0], qkv[1], qkv[2]
        scores = jnp.einsum("bhqd,bhkd->bhqk", q, k) * (Dh ** -0.5)
        idx = jnp.arange(S)
        mask = (idx[:, None] - idx[None, :] >= 0) & (idx[:, None] - idx[None, :] < W)
        scores = jnp.where(mask[None, None], scores, -1e9)
        p = _softmax(scores, axis=-1)
        o = jnp.einsum("bhqk,bhkd->bhqd", p, v)
        return (lambda x, *d: x.transpose(*d))(o, 0, 2, 1, 3).reshape(B, S, D) @ wo

    def _B_ref(x, w1, w2):
        h = jnp.einsum("bsd,df->bsf", x, w1)
        h = _silu(h)
        out = jnp.einsum("bsf,fd->bsd", h, w2)
        return out

    x = A_x
    g = _sigmoid((x * gate_w).sum(-1, keepdims=True))
    a = _A_ref(x, A_wqkv, A_wo)
    b = _B_ref(x, B_w1, B_w2)
    return g * a + (1 - g) * b
```

```python
import functools

import jax
import jax.numpy as jnp
import jax.experimental.pallas as pl
import jax.experimental.pallas.tpu as pltpu

S = 2048
D = 640
F = 1536
H = 32
DH = 20
W = 256
TB = 256
QB = 128
NEG = -1e30

_NT = (((1,), (1,)), ((), ()))
_TN = (((0,), (0,)), ((), ()))


def _head_tiles(h):
    lo, hi = DH * h, DH * h + DH
    t0, t1 = lo // 128, (hi - 1) // 128
    return t0, t1


def _attn_subblock(q_s, k_s, vt_s, ot_s, qoff, koff, nblk):
    f32 = jnp.float32
    bf16 = jnp.bfloat16
    row = jax.lax.broadcasted_iota(jnp.int32, (QB, QB), 0)
    col = jax.lax.broadcasted_iota(jnp.int32, (QB, QB), 1)
    tri = row <= col
    nk = nblk * QB
    kstart = koff - (nblk - 1) * QB
    sub = jax.lax.broadcasted_iota(jnp.int32, (8, QB), 0)

    outs = []
    for h in range(H):
        t0, t1 = _head_tiles(h)
        wl = (t1 - t0 + 1) * 128
        lane = jax.lax.broadcasted_iota(jnp.int32, (QB, wl), 1) + t0 * 128
        hm = (lane >= DH * h) & (lane < DH * h + DH)
        q = q_s[pl.ds(qoff, QB), t0 * 128:t0 * 128 + wl]
        qm = jnp.where(hm, q, jnp.zeros_like(q))
        k = k_s[pl.ds(kstart, nk), t0 * 128:t0 * 128 + wl]
        st = jax.lax.dot_general(k, qm, _NT, preferred_element_type=f32)
        sd = st[(nblk - 1) * QB:]
        if nblk == 3:
            t = jnp.where(tri, sd, st[:QB])
        else:
            t = jnp.where(tri, sd, NEG)
        m = jnp.max(t, axis=0, keepdims=True)
        if nblk >= 2:
            sm = st[(nblk - 2) * QB:(nblk - 1) * QB]
            m = jnp.maximum(m, jnp.max(sm, axis=0, keepdims=True))
        e = jnp.exp(t - m)
        l = jnp.sum(e, axis=0, keepdims=True)
        parts = []
        if nblk == 3:
            parts.append(jnp.where(tri, 0.0, e).astype(bf16))
        if nblk >= 2:
            em = jnp.exp(sm - m)
            l = l + jnp.sum(em, axis=0, keepdims=True)
            parts.append(em.astype(bf16))
        if nblk == 3:
            parts.append(jnp.where(tri, e, 0.0).astype(bf16))
        else:
            parts.append(e.astype(bf16))
        pt = jnp.concatenate(parts, axis=0) if len(parts) > 1 else parts[0]
        ws = 16 * ((DH * h) // 16)
        vt = vt_s[ws:ws + 32, pl.ds(kstart, nk)]
        o = jnp.dot(vt, pt, preferred_element_type=f32)
        o = o * (1.0 / l)
        outs.append(o)

    for g4 in range(H // 4):
        o0, o1, o2, o3 = outs[4 * g4:4 * g4 + 4]
        lo4 = sub < 4
        blk = jnp.concatenate([
            o0[0:16],
            jnp.where(lo4, o0[16:24], o1[0:8]),
            o1[8:24],
            o2[8:24],
            jnp.where(lo4, o2[24:32], o3[8:16]),
            o3[16:32],
        ], axis=0)
        ot_s[80 * g4:80 * g4 + 80, pl.ds(qoff, QB)] = blk.astype(bf16)


def _kernel(x_ref, wqkv_ref, wo_ref, w1_ref, w2_ref, gw_ref, o_ref,
            k_s, vt_s, wvt_s, q_s, ot_s):
    f32 = jnp.float32
    bf16 = jnp.bfloat16
    i = pl.program_id(0)

    @pl.when(i == 0)
    def _():
        wvt_s[...] = wqkv_ref[:, 2 * D:3 * D].T

    x = x_ref[...]
    base = pl.multiple_of(i * TB, TB)
    qk = jnp.dot(x, wqkv_ref[:, :2 * D], preferred_element_type=f32)
    q_s[...] = (qk[:, :D] * (DH ** -0.5)).astype(bf16)
    k_s[pl.ds(base, TB), :] = qk[:, D:].astype(bf16)
    vt = jax.lax.dot_general(wvt_s[...], x, _NT, preferred_element_type=f32)
    vt_s[:, pl.ds(base, TB)] = vt.astype(bf16)

    @pl.when(i == 0)
    def _():
        _attn_subblock(q_s, k_s, vt_s, ot_s, 0, 0, 1)
        _attn_subblock(q_s, k_s, vt_s, ot_s, QB, QB, 2)
        for sb in range(2, TB // QB):
            _attn_subblock(q_s, k_s, vt_s, ot_s, sb * QB, sb * QB, 3)

    @pl.when(i > 0)
    def _():
        def body(sb, carry):
            qoff = pl.multiple_of(sb * QB, QB)
            koff = pl.multiple_of(base + sb * QB, QB)
            _attn_subblock(q_s, k_s, vt_s, ot_s, qoff, koff, 3)
            return carry
        jax.lax.fori_loop(0, TB // QB, body, 0)

    a = jax.lax.dot_general(ot_s[...], wo_ref[...], _TN, preferred_element_type=f32)
    hmid = jnp.dot(x, w1_ref[...], preferred_element_type=f32)
    hmid = hmid * jax.nn.sigmoid(hmid)
    b = jnp.dot(hmid.astype(bf16), w2_ref[...], preferred_element_type=f32)
    gl = jnp.sum(x.astype(f32) * gw_ref[...].astype(f32), axis=-1, keepdims=True)
    g = jax.nn.sigmoid(gl)
    o_ref[...] = (g * a + (1.0 - g) * b).astype(o_ref.dtype)


@jax.jit
def pallas_gated_mix__sliding_block__dense_activation_silu__prompt_kernel(
    A_x: jax.Array,
    A_wqkv: jax.Array,
    A_wo: jax.Array,
    B_x: jax.Array,
    B_w1: jax.Array,
    B_w2: jax.Array,
    gate_w: jax.Array,
):
    del B_x
    x = A_x.reshape(S, D)
    gw = gate_w.reshape(1, D)
    bf16 = jnp.bfloat16
    out = pl.pallas_call(
        _kernel,
        grid=(S // TB,),
        in_specs=[
            pl.BlockSpec((TB, D), lambda i: (i, 0)),
            pl.BlockSpec((D, 3 * D), lambda i: (0, 0)),
            pl.BlockSpec((D, D), lambda i: (0, 0)),
            pl.BlockSpec((D, F), lambda i: (0, 0)),
            pl.BlockSpec((F, D), lambda i: (0, 0)),
            pl.BlockSpec((1, D), lambda i: (0, 0)),
        ],
        out_specs=pl.BlockSpec((TB, D), lambda i: (i, 0)),
        out_shape=jax.ShapeDtypeStruct((S, D), bf16),
        scratch_shapes=[
            pltpu.VMEM((S, D), bf16),
            pltpu.VMEM((D, S), bf16),
            pltpu.VMEM((D, D), bf16),
            pltpu.VMEM((TB, D), bf16),
            pltpu.VMEM((D, TB), bf16),
        ],
        compiler_params=pltpu.CompilerParams(
            dimension_semantics=("arbitrary",),
            vmem_limit_bytes=100 * 1024 * 1024,
        ),
    )(x, A_wqkv, A_wo, B_w1, B_w2, gw)
    return out.reshape(1, S, D)
```

```python
import functools

import jax
import jax.numpy as jnp
import jax.experimental.pallas as pl
import jax.experimental.pallas.tpu as pltpu

S = 2048
D = 640
F = 1536
H = 32
DH = 20
W = 256
TB = 256
QB = 128
HB = QB // 2
NEG = -1e30
LOG2E = 1.4426950408889634
NT6 = 6

_NT = (((1,), (1,)), ((), ()))
_TN = (((0,), (0,)), ((), ()))

_STRADDLE = ((6, 0, 0), (12, 1, 64), (19, 2, 32), (25, 3, 96))


def _head_pos(h):
    lo, hi = DH * h, DH * h + DH
    if lo // 128 == (hi - 1) // 128:
        return lo // 128, lo % 128
    for hh, t, r in _STRADDLE:
        if hh == h:
            return 5, (lo % 128 + r) % 128
    raise AssertionError


def _tile_groups(t):
    if t == 5:
        return [[6, 19], [12, 25]]
    heads = [h for h in range(H) if _head_pos(h)[0] == t]
    return [heads[:3], heads[3:]]


def _lane_in(lane, start):
    end = start + DH
    if end <= 128:
        return (lane >= start) & (lane < end)
    return (lane >= start) | (lane < end - 128)


def _six_tiles(z):
    rows = z.shape[0]
    lane = jax.lax.broadcasted_iota(jnp.int32, (rows, 128), 1)
    tiles = [z[:, t * 128:(t + 1) * 128] for t in range(5)]
    parts = []
    for h, t, r in _STRADDLE:
        c = jnp.where(lane >= 64, tiles[t], tiles[t + 1])
        if r:
            c = pltpu.roll(c, r, 1)
        parts.append(c)
    s6 = parts[0]
    for (h, t, r), p in zip(_STRADDLE[1:], parts[1:]):
        s6 = jnp.where(_lane_in(lane, _head_pos(h)[1]), p, s6)
    return tiles + [s6]


def _attn_subblock(q_s, qr_s, k_s, kr_s, vt_s, ot_s, s_s, qoff, koff, nblk, fillers=()):
    f32 = jnp.float32
    bf16 = jnp.bfloat16
    row = jax.lax.broadcasted_iota(jnp.int32, (QB, QB), 0)
    col = jax.lax.broadcasted_iota(jnp.int32, (QB, QB), 1)
    tri = row <= col
    kstart = koff - (nblk - 1) * QB
    sub = jax.lax.broadcasted_iota(jnp.int32, (8, QB), 0)
    lane = jax.lax.broadcasted_iota(jnp.int32, (QB, 128), 1)
    laneh = jax.lax.broadcasted_iota(jnp.int32, (HB, 128), 1)

    slot = {}
    c0 = 0
    for t in range(NT6):
        groups = _tile_groups(t)
        heads = groups[0] + groups[1]
        ts = slice(t * 128, (t + 1) * 128)
        q = q_s[pl.ds(qoff, QB), ts]
        qs = [jnp.where(_lane_in(lane, _head_pos(h)[1]), q, 0.0).astype(bf16) for h in heads]
        qst = jnp.concatenate(qs, axis=0)
        for j, h in enumerate(heads):
            slot[h] = c0 + j
        cs = slice(c0 * QB, (c0 + len(heads)) * QB)
        if nblk == 3:
            k = k_s[pl.ds(kstart + HB, 2 * QB), ts]
            s_s[0:2 * QB, cs] = jax.lax.dot_general(k, qst, _NT, preferred_element_type=f32)
            khi = k_s[pl.ds(koff + HB, HB), ts]
            krlo = kr_s[pl.ds(kstart, HB), ts]
            qhi = q[HB:]
            qrlo = qr_s[pl.ds(qoff, HB), ts]
            cg = c0
            for g in groups:
                own = _lane_in(laneh, _head_pos(g[0])[1])
                for h in g[1:]:
                    own = own | _lane_in(laneh, _head_pos(h)[1])
                kd = jnp.where(own, khi, krlo)
                qd = []
                for h in g:
                    s0 = _head_pos(h)[1]
                    qd.append(jnp.where(_lane_in(laneh, (s0 + 64) % 128), qrlo, 0.0).astype(bf16))
                    qd.append(jnp.where(_lane_in(laneh, s0), qhi, 0.0).astype(bf16))
                qd = jnp.concatenate(qd, axis=0)
                s_s[2 * QB:2 * QB + HB, cg * QB:(cg + len(g)) * QB] = jax.lax.dot_general(
                    kd, qd, _NT, preferred_element_type=f32)
                cg += len(g)
        else:
            k = k_s[pl.ds(kstart, nblk * QB), ts]
            s_s[0:nblk * QB, cs] = jax.lax.dot_general(k, qst, _NT, preferred_element_type=f32)
        c0 += len(heads)

    outs = []
    fillers = list(fillers)
    every = H // max(len(fillers), 1)
    for h in range(H):
        if fillers and h % every == 0:
            fillers.pop(0)()
        cs = slice(slot[h] * QB, (slot[h] + 1) * QB)
        if nblk == 3:
            sdd = s_s[2 * QB:2 * QB + HB, cs]
            t = jnp.concatenate([
                jnp.where(tri[:HB], s_s[QB + HB:2 * QB, cs], sdd),
                jnp.where(tri[HB:], sdd, s_s[0:HB, cs]),
            ], axis=0)
            sm = s_s[HB:HB + QB, cs]
        else:
            t = jnp.where(tri, s_s[(nblk - 1) * QB:nblk * QB, cs], NEG)
            if nblk == 2:
                sm = s_s[0:QB, cs]
        m = jnp.max(t, axis=0, keepdims=True)
        if nblk >= 2:
            m = jnp.maximum(m, jnp.max(sm, axis=0, keepdims=True))
        e = jnp.exp2(t - m)
        l = jnp.sum(e, axis=0, keepdims=True)
        ws = 16 * ((DH * h) // 16)
        def pv(j, p):
            vt = vt_s[ws:ws + 32, pl.ds(kstart + j * QB, QB)]
            return jnp.dot(vt, p.astype(bf16), preferred_element_type=f32)
        if nblk == 3:
            o = pv(2, jnp.where(tri, e, 0.0)) + pv(0, jnp.where(tri, 0.0, e))
        else:
            o = pv(nblk - 1, e)
        if nblk >= 2:
            em = jnp.exp2(sm - m)
            l = l + jnp.sum(em, axis=0, keepdims=True)
            o = o + pv(nblk - 2, em)
        o = o * (1.0 / l)
        outs.append(o)

    for g4 in range(H // 4):
        o0, o1, o2, o3 = outs[4 * g4:4 * g4 + 4]
        lo4 = sub < 4
        blk = jnp.concatenate([
            o0[0:16],
            jnp.where(lo4, o0[16:24], o1[0:8]),
            o1[8:24],
            o2[8:24],
            jnp.where(lo4, o2[24:32], o3[8:16]),
            o3[16:32],
        ], axis=0)
        ot_s[80 * g4:80 * g4 + 80, pl.ds(qoff, QB)] = blk.astype(bf16)


def _kernel(x_ref, wqkv_hbm, wo_hbm, w1_hbm, w2_hbm, gw_ref, o_ref,
            k_s, kr_s, vt_s, wvt_s, q_s, qr_s, ot_s, s_s, h_s, b_s,
            wqk_ref, wv_ref, wo_ref, w1_ref, w2_ref, sems):
    f32 = jnp.float32
    bf16 = jnp.bfloat16
    i = pl.program_id(0)

    cp_qk = pltpu.make_async_copy(wqkv_hbm.at[:, 0:2 * D], wqk_ref, sems.at[0])
    cp_v = pltpu.make_async_copy(wqkv_hbm.at[:, 2 * D:3 * D], wv_ref, sems.at[1])
    cp_o = pltpu.make_async_copy(wo_hbm, wo_ref, sems.at[2])
    cp_1 = pltpu.make_async_copy(w1_hbm, w1_ref, sems.at[3])
    cp_2 = pltpu.make_async_copy(w2_hbm, w2_ref, sems.at[4])

    @pl.when(i == 0)
    def _():
        cp_v.start()
        cp_qk.start()
        cp_v.wait()
        wvt_s[...] = wv_ref[...].T
        cp_qk.wait()
        cp_o.start()
        cp_1.start()
        cp_2.start()

    def step_body(first):
        x = x_ref[...]
        base = 0 if first else pl.multiple_of(i * TB, TB)
        qk = jnp.dot(x, wqk_ref[...], preferred_element_type=f32)
        q6 = _six_tiles(qk[:, :D] * (DH ** -0.5 * LOG2E))
        k6 = _six_tiles(qk[:, D:])
        for t in range(NT6):
            ts = slice(t * 128, (t + 1) * 128)
            q_s[:, ts] = q6[t]
            k_s[pl.ds(base, TB), ts] = k6[t].astype(bf16)
            for sb in range(TB // QB):
                rs = slice(sb * QB, sb * QB + HB)
                qr_s[sb * QB:sb * QB + HB, ts] = pltpu.roll(q6[t][rs], 64, 1)
                kr_s[pl.ds(base + sb * QB, HB), ts] = pltpu.roll(k6[t][rs], 64, 1).astype(bf16)
        vt = jax.lax.dot_general(wvt_s[...], x, _NT, preferred_element_type=f32)
        vt_s[:, pl.ds(base, TB)] = vt.astype(bf16)

        NC1 = 4
        c1 = F // NC1
        def ffn1(c):
            def f():
                hm = jnp.dot(x, w1_ref[:, c * c1:(c + 1) * c1], preferred_element_type=f32)
                h_s[:, c * c1:(c + 1) * c1] = (hm * jax.nn.sigmoid(hm)).astype(bf16)
            return f
        def ffn2(c):
            def f():
                b_s[:, c * 128:(c + 1) * 128] = jnp.dot(
                    h_s[...], w2_ref[:, c * 128:(c + 1) * 128], preferred_element_type=f32)
            return f

        if first:
            for sb in range(TB // QB):
                nblk = min(sb + 1, 3)
                _attn_subblock(q_s, qr_s, k_s, kr_s, vt_s, ot_s, s_s.at[sb % 2],
                               sb * QB, base + sb * QB, nblk)
            cp_o.wait()
            cp_1.wait()
            cp_2.wait()
            for c in range(NC1):
                ffn1(c)()
            for c in range(5):
                ffn2(c)()
        else:
            _attn_subblock(q_s, qr_s, k_s, kr_s, vt_s, ot_s, s_s.at[0],
                           0, base, 3, [ffn1(c) for c in range(NC1)])
            _attn_subblock(q_s, qr_s, k_s, kr_s, vt_s, ot_s, s_s.at[1],
                           QB, base + QB, 3, [ffn2(c) for c in range(4)])
            ffn2(4)()

        a = jax.lax.dot_general(ot_s[...], wo_ref[...], _TN, preferred_element_type=f32)
        gl = jnp.sum(x.astype(f32) * gw_ref[...].astype(f32).reshape(1, D), axis=-1, keepdims=True)
        g = jax.nn.sigmoid(gl)
        o_ref[...] = (g * a + (1.0 - g) * b_s[...]).astype(o_ref.dtype)

    @pl.when(i == 0)
    def _():
        step_body(True)

    @pl.when(i > 0)
    def _():
        step_body(False)


@jax.jit
def pallas_gated_mix__sliding_block__dense_activation_silu__prompt_kernel(
    A_x: jax.Array,
    A_wqkv: jax.Array,
    A_wo: jax.Array,
    B_x: jax.Array,
    B_w1: jax.Array,
    B_w2: jax.Array,
    gate_w: jax.Array,
):
    del B_x
    x = A_x.reshape(S, D)
    gw = gate_w
    bf16 = jnp.bfloat16
    f32 = jnp.float32
    out = pl.pallas_call(
        _kernel,
        grid=(S // TB,),
        in_specs=[
            pl.BlockSpec((TB, D), lambda i: (i, 0)),
            pl.BlockSpec(memory_space=pl.ANY),
            pl.BlockSpec(memory_space=pl.ANY),
            pl.BlockSpec(memory_space=pl.ANY),
            pl.BlockSpec(memory_space=pl.ANY),
            pl.BlockSpec((D,), lambda i: (0,)),
        ],
        out_specs=pl.BlockSpec((TB, D), lambda i: (i, 0)),
        out_shape=jax.ShapeDtypeStruct((S, D), bf16),
        scratch_shapes=[
            pltpu.VMEM((S, NT6 * 128), bf16),
            pltpu.VMEM((S, NT6 * 128), bf16),
            pltpu.VMEM((D, S), bf16),
            pltpu.VMEM((D, D), bf16),
            pltpu.VMEM((TB, NT6 * 128), f32),
            pltpu.VMEM((TB, NT6 * 128), f32),
            pltpu.VMEM((D, TB), bf16),
            pltpu.VMEM((2, 3 * QB, H * QB), f32),
            pltpu.VMEM((TB, F), bf16),
            pltpu.VMEM((TB, D), f32),
            pltpu.VMEM((D, 2 * D), bf16),
            pltpu.VMEM((D, D), bf16),
            pltpu.VMEM((D, D), bf16),
            pltpu.VMEM((D, F), bf16),
            pltpu.VMEM((F, D), bf16),
            pltpu.SemaphoreType.DMA((5,)),
        ],
        compiler_params=pltpu.CompilerParams(
            dimension_semantics=("arbitrary",),
            vmem_limit_bytes=100 * 1024 * 1024,
        ),
    )(x, A_wqkv, A_wo, B_w1, B_w2, gw)
    return out.reshape(1, S, D)
```

```python
import jax
import jax.numpy as jnp
import jax.experimental.pallas as pl
import jax.experimental.pallas.tpu as pltpu

S = 2048
D = 640
F = 1536
H = 32
DH = 20
W = 256
TB = 256
QB = 128
HB = QB // 2
NEG = -1e30
LOG2E = 1.4426950408889634
SPAN = 28
NT6 = 6

_NT = (((1,), (1,)), ((), ()))
_TN = (((0,), (0,)), ((), ()))

_STRADDLE = ((6, 0, 0), (12, 1, 64), (19, 2, 32), (25, 3, 96))


def _head_pos(h):
    lo, hi = DH * h, DH * h + DH
    if lo // 128 == (hi - 1) // 128:
        return lo // 128, lo % 128
    for hh, t, r in _STRADDLE:
        if hh == h:
            return 5, (lo % 128 + r) % 128
    raise AssertionError


def _tile_groups(t):
    if t == 5:
        return [[6, 19], [12, 25]]
    heads = [h for h in range(H) if _head_pos(h)[0] == t]
    return [heads[:3], heads[3:]]


def _lane_in(lane, start):
    end = start + DH
    if end <= 128:
        return (lane >= start) & (lane < end)
    return (lane >= start) | (lane < end - 128)


def _six_tiles(z):
    rows = z.shape[0]
    lane = jax.lax.broadcasted_iota(jnp.int32, (rows, 128), 1)
    tiles = [z[:, t * 128:(t + 1) * 128] for t in range(5)]
    parts = []
    for h, t, r in _STRADDLE:
        c = jnp.where(lane >= 64, tiles[t], tiles[t + 1])
        if r:
            c = pltpu.roll(c, r, 1)
        parts.append(c)
    s6 = parts[0]
    for (h, t, r), p in zip(_STRADDLE[1:], parts[1:]):
        s6 = jnp.where(_lane_in(lane, _head_pos(h)[1]), p, s6)
    return tiles + [s6]


def _attn_subblock(q_s, qr_s, k_s, kr_s, vt_s, ot_s, s_s, qoff, koff, nblk, fillers=()):
    f32 = jnp.float32
    bf16 = jnp.bfloat16
    row = jax.lax.broadcasted_iota(jnp.int32, (QB, QB), 0)
    col = jax.lax.broadcasted_iota(jnp.int32, (QB, QB), 1)
    tri = row <= col
    kstart = koff - (nblk - 1) * QB
    sub = jax.lax.broadcasted_iota(jnp.int32, (8, QB), 0)
    lane = jax.lax.broadcasted_iota(jnp.int32, (QB, 128), 1)
    laneh = jax.lax.broadcasted_iota(jnp.int32, (HB, 128), 1)

    slot = {}
    c0 = 0
    for t in range(NT6):
        groups = _tile_groups(t)
        heads = groups[0] + groups[1]
        ts = slice(t * 128, (t + 1) * 128)
        q = q_s[pl.ds(qoff, QB), ts]
        qs = [jnp.where(_lane_in(lane, _head_pos(h)[1]), q, 0.0).astype(bf16) for h in heads]
        qst = jnp.concatenate(qs, axis=0)
        for j, h in enumerate(heads):
            slot[h] = c0 + j
        cs = slice(c0 * QB, (c0 + len(heads)) * QB)
        if nblk == 3:
            k = k_s[pl.ds(kstart + HB, 2 * QB), ts]
            s_s[0:2 * QB, cs] = jax.lax.dot_general(k, qst, _NT, preferred_element_type=f32)
            khi = k_s[pl.ds(koff + HB, HB), ts]
            krlo = kr_s[pl.ds(kstart, HB), ts]
            qhi = q[HB:]
            qrlo = qr_s[pl.ds(qoff, HB), ts]
            cg = c0
            for g in groups:
                own = _lane_in(laneh, _head_pos(g[0])[1])
                for h in g[1:]:
                    own = own | _lane_in(laneh, _head_pos(h)[1])
                kd = jnp.where(own, khi, krlo)
                qd = []
                for h in g:
                    s0 = _head_pos(h)[1]
                    qd.append(jnp.where(_lane_in(laneh, (s0 + 64) % 128), qrlo, 0.0).astype(bf16))
                    qd.append(jnp.where(_lane_in(laneh, s0), qhi, 0.0).astype(bf16))
                qd = jnp.concatenate(qd, axis=0)
                s_s[2 * QB:2 * QB + HB, cg * QB:(cg + len(g)) * QB] = jax.lax.dot_general(
                    kd, qd, _NT, preferred_element_type=f32)
                cg += len(g)
        else:
            k = k_s[pl.ds(kstart, nblk * QB), ts]
            s_s[0:nblk * QB, cs] = jax.lax.dot_general(k, qst, _NT, preferred_element_type=f32)
        c0 += len(heads)

    outs = []
    fillers = list(fillers)
    nf = len(fillers)
    pos = [(c * SPAN) // nf for c in range(nf)]
    for h in range(H):
        while fillers and pos[nf - len(fillers)] <= h:
            fillers.pop(0)()
        cs = slice(slot[h] * QB, (slot[h] + 1) * QB)
        if nblk == 3:
            sdd = s_s[2 * QB:2 * QB + HB, cs]
            t = jnp.concatenate([
                jnp.where(tri[:HB], s_s[QB + HB:2 * QB, cs], sdd),
                jnp.where(tri[HB:], sdd, s_s[0:HB, cs]),
            ], axis=0)
            sm = s_s[HB:HB + QB, cs]
        else:
            t = jnp.where(tri, s_s[(nblk - 1) * QB:nblk * QB, cs], NEG)
            if nblk == 2:
                sm = s_s[0:QB, cs]
        m = jnp.max(t, axis=0, keepdims=True)
        if nblk >= 2:
            m = jnp.maximum(m, jnp.max(sm, axis=0, keepdims=True))
        e = jnp.exp2(t - m)
        l = jnp.sum(e, axis=0, keepdims=True)
        ws = 16 * ((DH * h) // 16)
        def pv(j, p):
            vt = vt_s[ws:ws + 32, pl.ds(kstart + j * QB, QB)]
            return jnp.dot(vt, p.astype(bf16), preferred_element_type=f32)
        if nblk == 3:
            o = pv(2, jnp.where(tri, e, 0.0)) + pv(0, jnp.where(tri, 0.0, e))
        else:
            o = pv(nblk - 1, e)
        if nblk >= 2:
            em = jnp.exp2(sm - m)
            l = l + jnp.sum(em, axis=0, keepdims=True)
            o = o + pv(nblk - 2, em)
        o = o * (1.0 / l)
        outs.append(o)

    for g4 in range(H // 4):
        o0, o1, o2, o3 = outs[4 * g4:4 * g4 + 4]
        lo4 = sub < 4
        blk = jnp.concatenate([
            o0[0:16],
            jnp.where(lo4, o0[16:24], o1[0:8]),
            o1[8:24],
            o2[8:24],
            jnp.where(lo4, o2[24:32], o3[8:16]),
            o3[16:32],
        ], axis=0)
        ot_s[80 * g4:80 * g4 + 80, pl.ds(qoff, QB)] = blk.astype(bf16)


def _kernel(x_ref, wqkv_hbm, wo_hbm, w1_hbm, w2_hbm, gw_ref, o_ref,
            k_s, kr_s, vt_s, wvt_s, q_s, qr_s, ot_s, s_s, h_s, b_s,
            wqk_ref, wv_ref, wo_ref, w1_ref, w2_ref, sems):
    f32 = jnp.float32
    bf16 = jnp.bfloat16
    i = pl.program_id(0)

    cp_qk = pltpu.make_async_copy(wqkv_hbm.at[:, 0:2 * D], wqk_ref, sems.at[0])
    cp_v = pltpu.make_async_copy(wqkv_hbm.at[:, 2 * D:3 * D], wv_ref, sems.at[1])
    cp_o = pltpu.make_async_copy(wo_hbm, wo_ref, sems.at[2])
    cp_1 = pltpu.make_async_copy(w1_hbm, w1_ref, sems.at[3])
    cp_2 = pltpu.make_async_copy(w2_hbm, w2_ref, sems.at[4])

    @pl.when(i == 0)
    def _():
        cp_v.start()
        cp_qk.start()
        cp_v.wait()
        wvt_s[...] = wv_ref[...].T
        cp_qk.wait()
        cp_1.start()
        cp_2.start()
        cp_o.start()

    def step_body(first):
        x = x_ref[...]
        base = 0 if first else pl.multiple_of(i * TB, TB)
        qk = jnp.dot(x, wqk_ref[...], preferred_element_type=f32)
        q6 = _six_tiles(qk[:, :D] * (DH ** -0.5 * LOG2E))
        k6 = _six_tiles(qk[:, D:])
        for t in range(NT6):
            ts = slice(t * 128, (t + 1) * 128)
            q_s[:, ts] = q6[t]
            k_s[pl.ds(base, TB), ts] = k6[t].astype(bf16)
            for sb in range(TB // QB):
                rs = slice(sb * QB, sb * QB + HB)
                qr_s[sb * QB:sb * QB + HB, ts] = pltpu.roll(q6[t][rs], 64, 1)
                kr_s[pl.ds(base + sb * QB, HB), ts] = pltpu.roll(k6[t][rs], 64, 1).astype(bf16)
        vt = jax.lax.dot_general(wvt_s[...], x, _NT, preferred_element_type=f32)
        vt_s[:, pl.ds(base, TB)] = vt.astype(bf16)

        NC1 = 12
        c1 = F // NC1
        def ffn1(c):
            def f():
                hm = jnp.dot(x, w1_ref[:, c * c1:(c + 1) * c1], preferred_element_type=f32)
                h_s[:, c * c1:(c + 1) * c1] = (hm * jax.nn.sigmoid(hm)).astype(bf16)
            return f
        def ffn2(c, mh=None):
            def f():
                rs = slice(0, TB) if mh is None else slice(mh * QB, (mh + 1) * QB)
                b_s[rs, c * 128:(c + 1) * 128] = jnp.dot(
                    h_s[rs, :], w2_ref[:, c * 128:(c + 1) * 128], preferred_element_type=f32)
            return f

        if first:
            _attn_subblock(q_s, qr_s, k_s, kr_s, vt_s, ot_s, s_s.at[0], 0, 0, 1)
            cp_1.wait()
            _attn_subblock(q_s, qr_s, k_s, kr_s, vt_s, ot_s, s_s.at[1], QB, QB, 2,
                           [ffn1(c) for c in range(NC1)])
            cp_o.wait()
            cp_2.wait()
            for c in range(5):
                ffn2(c)()
        else:
            _attn_subblock(q_s, qr_s, k_s, kr_s, vt_s, ot_s, s_s.at[0],
                           0, base, 3, [ffn1(c) for c in range(NC1)])
            _attn_subblock(q_s, qr_s, k_s, kr_s, vt_s, ot_s, s_s.at[1],
                           QB, base + QB, 3, [ffn2(c, mh) for c in range(4) for mh in range(2)])
            ffn2(4)()

        a = jax.lax.dot_general(ot_s[...], wo_ref[...], _TN, preferred_element_type=f32)
        gl = jnp.sum(x.astype(f32) * gw_ref[...].astype(f32).reshape(1, D), axis=-1, keepdims=True)
        g = jax.nn.sigmoid(gl)
        o_ref[...] = (g * a + (1.0 - g) * b_s[...]).astype(o_ref.dtype)

    @pl.when(i == 0)
    def _():
        step_body(True)

    @pl.when(i > 0)
    def _():
        step_body(False)


@jax.jit
def pallas_gated_mix__sliding_block__dense_activation_silu__prompt_kernel(
    A_x: jax.Array,
    A_wqkv: jax.Array,
    A_wo: jax.Array,
    B_x: jax.Array,
    B_w1: jax.Array,
    B_w2: jax.Array,
    gate_w: jax.Array,
):
    del B_x
    x = A_x.reshape(S, D)
    gw = gate_w
    bf16 = jnp.bfloat16
    f32 = jnp.float32
    out = pl.pallas_call(
        _kernel,
        grid=(S // TB,),
        in_specs=[
            pl.BlockSpec((TB, D), lambda i: (i, 0)),
            pl.BlockSpec(memory_space=pl.ANY),
            pl.BlockSpec(memory_space=pl.ANY),
            pl.BlockSpec(memory_space=pl.ANY),
            pl.BlockSpec(memory_space=pl.ANY),
            pl.BlockSpec((D,), lambda i: (0,)),
        ],
        out_specs=pl.BlockSpec((TB, D), lambda i: (i, 0)),
        out_shape=jax.ShapeDtypeStruct((S, D), bf16),
        scratch_shapes=[
            pltpu.VMEM((S, NT6 * 128), bf16),
            pltpu.VMEM((S, NT6 * 128), bf16),
            pltpu.VMEM((D, S), bf16),
            pltpu.VMEM((D, D), bf16),
            pltpu.VMEM((TB, NT6 * 128), f32),
            pltpu.VMEM((TB, NT6 * 128), f32),
            pltpu.VMEM((D, TB), bf16),
            pltpu.VMEM((2, 3 * QB, H * QB), f32),
            pltpu.VMEM((TB, F), bf16),
            pltpu.VMEM((TB, D), f32),
            pltpu.VMEM((D, 2 * D), bf16),
            pltpu.VMEM((D, D), bf16),
            pltpu.VMEM((D, D), bf16),
            pltpu.VMEM((D, F), bf16),
            pltpu.VMEM((F, D), bf16),
            pltpu.SemaphoreType.DMA((5,)),
        ],
        compiler_params=pltpu.CompilerParams(
            dimension_semantics=("arbitrary",),
            vmem_limit_bytes=100 * 1024 * 1024,
        ),
    )(x, A_wqkv, A_wo, B_w1, B_w2, gw)
    return out.reshape(1, S, D)
```
